```python
import os as _os
_os.environ.setdefault("JAX_PLATFORMS", "cpu")
import jax
import jax.numpy as jnp

def _softmax(x, axis=-1):
    return jax.nn.softmax(x, axis=axis)
def _gelu(x):
    return jax.nn.gelu(x, approximate=True)
def _silu(x):
    return jax.nn.silu(x)
def _sigmoid(x):
    return jax.nn.sigmoid(x)
def _layernorm(x, axis=-1, eps=1e-5):
    m = jnp.mean(x, axis=axis, keepdims=True)
    v = jnp.var(x, axis=axis, keepdims=True)
    return (x - m) / jnp.sqrt(v + eps)
def _scatter_add(tgt, idx, src, axis=0):
    return tgt.at[idx].add(src)
def _segment_sum(src, seg, n):
    return jax.ops.segment_sum(src, seg, n)
class _Rng:
    def __init__(self, key):
        self._k = key
    def _next(self):
        self._k, sub = jax.random.split(self._k)
        return sub
    def normal(self, shape):
        return jax.random.normal(self._next(), shape, dtype=jnp.bfloat16)
    def randint(self, lo, hi, shape):
        return jax.random.randint(self._next(), shape, lo, hi, dtype=jnp.int32)
    def uniform(self, shape, lo=0.0, hi=1.0):
        return jax.random.uniform(self._next(), shape, jnp.bfloat16, lo, hi)
    def permutation(self, n):
        return jax.random.permutation(self._next(), n)


kernel_name = 'standalone__detection_seg_fpn_lateral__vision'

def setup_inputs():
    _rng = _Rng(jax.random.key(int.from_bytes(__import__("os").urandom(4), "little")))
    _w = (lambda a: (lambda t: t.astype(jnp.bfloat16) if jnp.issubdtype(t.dtype, jnp.floating) else t)(jnp.asarray(a)))
    H = W = (256 // 2) * 2
    C = 384
    k = 1
    return {
        "c_fine": _w((lambda *s: _rng.normal(s) * 0.05)(1, H, W, C)),
        "p_coarse": _w((lambda *s: _rng.normal(s) * 0.05)(1, H // 2, W // 2, C)),
        "w_lat": _w((lambda *s: _rng.normal(s) * 0.05)(C, C)),
        "w_out": _w((lambda *s: _rng.normal(s) * 0.05)(k, k, C, C)),
    }

def reference(c_fine, p_coarse, w_lat, w_out):
    B, H, W, C = c_fine.shape
    k = 1
    lat = jnp.einsum("bhwc,cd->bhwd", c_fine, w_lat)
    up = jnp.repeat(jnp.repeat(p_coarse, 2, axis=1), 2, axis=2)
    m = lat + up
    pad = k // 2
    mp = jnp.pad(m, ((0, 0), (pad, pad), (pad, pad), (0, 0)))
    o = None
    for di in range(k):
        for dj in range(k):
            t = jnp.einsum("bhwc,cd->bhwd", mp[:, di:di + H, dj:dj + W, :], w_out[di, dj])
            o = t if o is None else o + t
    return o
```

```python
import jax
import jax.numpy as jnp
from jax import lax
import jax.experimental.pallas as pl
import jax.experimental.pallas.tpu as pltpu

_F32 = jnp.float32
_BF16 = jnp.bfloat16

_STREAMS = 8
_STRIDE = 1024
_PIECE = 32
_SWITCH = 18
_INIT = 3


@jax.jit
def pallas_standalone__detection_seg_fpn_lateral__vision_kernel(
    c_fine: jax.Array,
    p_coarse: jax.Array,
    w_lat: jax.Array,
    w_out: jax.Array,
):
    B, H, W, C = c_fine.shape
    assert (B, H, W, C) == (1, 256, 256, 384)
    n_fine = H * W
    pair = 2 * W
    wc = W // 2
    n_pair = n_fine // pair
    n_group = n_fine // _STRIDE
    spg = _STRIDE // pair
    n_slab = n_pair // _STREAMS
    half = _STREAMS // 2
    n_step = 2 * n_slab
    n_piece = pair // _PIECE

    def kernel(c_hbm, p_hbm, wl_hbm, wo_hbm, o_hbm,
               cbuf, pbuf, obuf, wl_ref, wo_ref, wc_ref, rsem, osem):
        def c_in(i):
            sl, j = i // 2, i % 2
            sb, s = sl // spg, sl % spg
            return pltpu.make_async_copy(
                c_hbm.at[pl.ds(_STREAMS * sb + half * j, half), pl.ds(s * pair, pair), :],
                cbuf.at[pl.ds(half * i, half)], rsem.at[i])

        def p_in(sl):
            sb, s = sl // spg, sl % spg
            return pltpu.make_async_copy(
                p_hbm.at[pl.ds(_STREAMS * sb, _STREAMS), pl.ds(s * wc, wc), :],
                pbuf.at[pl.ds(_STREAMS * sl, _STREAMS)], rsem.at[n_step + sl])

        def o_start(sl):
            sb, s = sl // spg, sl % spg
            for k in range(n_piece):
                pltpu.make_async_copy(
                    obuf.at[pl.ds(_STREAMS * sl, _STREAMS), pl.ds(k * _PIECE, _PIECE), :],
                    o_hbm.at[pl.ds(_STREAMS * sb, _STREAMS),
                             pl.ds(s * pair + k * _PIECE, _PIECE), :],
                    osem.at[0]).start()

        wl_cp = pltpu.make_async_copy(wl_hbm, wl_ref, rsem.at[n_step + n_slab])
        wo_cp = pltpu.make_async_copy(wo_hbm, wo_ref, rsem.at[n_step + n_slab + 1])
        wl_cp.start()
        wo_cp.start()
        for sl in range(n_slab):
            p_in(sl).start()
            c_in(2 * sl).start()
            c_in(2 * sl + 1).start()
        wl_cp.wait()
        wo_cp.wait()
        wc_ref[...] = jnp.dot(
            wl_ref[...], wo_ref[...], preferred_element_type=_F32).astype(_BF16)

        def step(i, carry):
            @pl.when(i <= _SWITCH)
            def _():
                @pl.when(i % 2 == 0)
                def _():
                    p_in(i // 2).wait()
                c_in(i).wait()

            p = pbuf[pl.ds(half * i, half)].reshape(half * wc, C)
            q = jnp.dot(p, wo_ref[...], preferred_element_type=_F32)
            qq = pltpu.pack_elementwise([q, q], packed_dtype=_BF16)
            qup = pltpu.bitcast(qq, _BF16).astype(_F32)
            c = cbuf[pl.ds(half * i, half)].reshape(half * pair, C)
            y = jnp.dot(c, wc_ref[...], preferred_element_type=_F32)
            y = y.reshape(half, 2, W, C) + qup.reshape(half, 1, W, C)
            obuf[pl.ds(half * i, half)] = y.reshape(half, pair, C).astype(_BF16)

            @pl.when(i == _SWITCH)
            def _():
                for ii in range(_SWITCH + 1, n_step):
                    if ii % 2 == 0:
                        p_in(ii // 2).wait()
                    c_in(ii).wait()
                for sl in range(_INIT):
                    o_start(sl)

            @pl.when(i > _SWITCH)
            def _():
                o_start(i - (_SWITCH + 1) + _INIT)

            return carry

        lax.fori_loop(0, n_step, step, 0)
        issued = _INIT + (n_step - 1 - _SWITCH)
        for sl in range(issued, n_slab):
            o_start(sl)
        pltpu.make_async_copy(obuf, obuf, osem.at[0]).wait()

    any_spec = pl.BlockSpec(memory_space=pl.ANY)
    out = pl.pallas_call(
        kernel,
        in_specs=[any_spec] * 4,
        out_specs=any_spec,
        out_shape=jax.ShapeDtypeStruct((n_group, _STRIDE, C), _BF16),
        scratch_shapes=[
            pltpu.VMEM((n_pair, pair, C), _BF16),
            pltpu.VMEM((n_pair, wc, C), _BF16),
            pltpu.VMEM((n_pair, pair, C), _BF16),
            pltpu.VMEM((C, C), _BF16),
            pltpu.VMEM((C, C), _BF16),
            pltpu.VMEM((C, C), _BF16),
            pltpu.SemaphoreType.DMA((n_step + n_slab + 2,)),
            pltpu.SemaphoreType.DMA((1,)),
        ],
        compiler_params=pltpu.CompilerParams(vmem_limit_bytes=124 * 1024 * 1024),
    )(
        c_fine.reshape(n_group, _STRIDE, C),
        p_coarse.reshape(n_group, _STRIDE // 4, C),
        w_lat,
        w_out.reshape(C, C),
    )
    return out.reshape(B, H, W, C)
```

```python
import jax
import jax.numpy as jnp
from jax import lax
import jax.experimental.pallas as pl
import jax.experimental.pallas.tpu as pltpu

_F32 = jnp.float32
_BF16 = jnp.bfloat16
_LANES = 128

_STREAMS = 8
_STRIDE = 4096
_PIECE = 32
_SWITCH = 18
_INIT = 3
_TAIL = 160


@jax.jit
def pallas_standalone__detection_seg_fpn_lateral__vision_kernel(
    c_fine: jax.Array,
    p_coarse: jax.Array,
    w_lat: jax.Array,
    w_out: jax.Array,
):
    B, H, W, C = c_fine.shape
    assert (B, H, W, C) == (1, 256, 256, 384) and w_out.shape == (1, 1, C, C)
    n_fine = H * W
    pair = 2 * W
    wc = W // 2
    n_pair = n_fine // pair
    n_group = n_fine // _STRIDE
    spg = _STRIDE // pair
    n_slab = n_pair // _STREAMS
    half = _STREAMS // 2
    n_step = 2 * n_slab
    n_q = half * wc
    last = n_step - 1
    sem_p, sem_w, sem_tail = n_step, n_step + n_slab, n_step + n_slab + 2
    n_issued = _INIT + (last - _SWITCH)
    assert 2 * _INIT <= _SWITCH + 1 and n_issued <= n_slab
    assert all(2 * (i - _SWITCH - 1 + _INIT) + 1 <= i for i in range(_SWITCH + 1, n_step))

    def kernel(c_hbm, p_hbm, wl_hbm, wo_hbm, o_hbm,
               xbuf, pbuf, wl_ref, wo_ref, wf_ref, qup_ref, osem):
        def start_out(sl):
            g0, r0 = (sl // spg) * _STREAMS, (sl % spg) * pair
            for k in range(pair // _PIECE):
                pltpu.make_async_copy(
                    xbuf.at[pl.ds(_STREAMS * sl, _STREAMS), pl.ds(k * _PIECE, _PIECE), :],
                    o_hbm.at[pl.ds(g0, _STREAMS), pl.ds(r0 + k * _PIECE, _PIECE), :],
                    osem.at[0]).start()

        def main(rsem):
            def c_in(i, lo=0, size=pair, sem=None):
                sl = i // 2
                g0, r0 = (sl // spg) * _STREAMS + (i % 2) * half, (sl % spg) * pair
                return pltpu.make_async_copy(
                    c_hbm.at[pl.ds(g0, half), pl.ds(r0 + lo, size), :],
                    xbuf.at[pl.ds(half * i, half), pl.ds(lo, size), :],
                    rsem.at[i if sem is None else sem])

            def p_in(sl):
                g0, r0 = (sl // spg) * _STREAMS, (sl % spg) * wc
                return pltpu.make_async_copy(
                    p_hbm.at[pl.ds(g0, _STREAMS), pl.ds(r0, wc), :],
                    pbuf.at[pl.ds(_STREAMS * sl, _STREAMS)],
                    rsem.at[sem_p + sl])

            def c_last_head():
                return c_in(last, 0, pair - _TAIL)

            def c_last_tail():
                return c_in(last, pair - _TAIL, _TAIL, sem_tail)

            wl_in = pltpu.make_async_copy(wl_hbm, wl_ref, rsem.at[sem_w])
            wo_in = pltpu.make_async_copy(wo_hbm, wo_ref, rsem.at[sem_w + 1])
            wl_in.start()
            wo_in.start()
            for i in range(last):
                if i % 2 == 0:
                    p_in(i // 2).start()
                c_in(i).start()
            c_last_head().start()
            c_last_tail().start()

            wl_in.wait()
            wo_in.wait()
            wf_ref[...] = jnp.dot(
                wl_ref[...], wo_ref[...], preferred_element_type=_F32).astype(_BF16)

            def step(i, carry):
                @pl.when(i <= _SWITCH)
                def _():
                    @pl.when(i % 2 == 0)
                    def _():
                        p_in(i // 2).wait()

                    c_in(i).wait()

                rows = pl.ds(half * i, half)
                q = jnp.dot(pbuf[rows].reshape(n_q, C), wo_ref[...],
                            preferred_element_type=_F32)
                for j in range(C // _LANES):
                    qj = q[:, j * _LANES:(j + 1) * _LANES]
                    qup_ref[j, pl.ds(0, n_q, stride=2), :] = qj
                    qup_ref[j, pl.ds(1, n_q, stride=2), :] = qj
                qup = jnp.concatenate(
                    [qup_ref[j, pl.ds(0, 2 * n_q), :] for j in range(C // _LANES)], axis=1)
                y = jnp.dot(xbuf[rows].reshape(half * pair, C), wf_ref[...],
                            preferred_element_type=_F32)
                y = y.reshape(half, 2, W, C) + qup.reshape(half, 1, W, C)
                xbuf[rows] = y.reshape(half, pair, C).astype(_BF16)

                @pl.when(i == _SWITCH)
                def _():
                    for ii in range(_SWITCH + 1, last):
                        if ii % 2 == 0:
                            p_in(ii // 2).wait()
                        c_in(ii).wait()
                    c_last_head().wait()
                    for sl in range(_INIT):
                        start_out(sl)
                    c_last_tail().wait()

                @pl.when(i > _SWITCH)
                def _():
                    start_out(i - (_SWITCH + 1) + _INIT)

                return carry

            lax.fori_loop(0, n_step, step, 0)
            for sl in range(n_issued, n_slab):
                start_out(sl)

        pl.run_scoped(main, pltpu.SemaphoreType.DMA((sem_tail + 1,)))
        pltpu.make_async_copy(o_hbm, o_hbm, osem.at[0]).wait()

    any_spec = pl.BlockSpec(memory_space=pl.ANY)
    out = pl.pallas_call(
        kernel,
        in_specs=[any_spec] * 4,
        out_specs=any_spec,
        out_shape=jax.ShapeDtypeStruct((n_group, _STRIDE, C), _BF16),
        scratch_shapes=[
            pltpu.VMEM((n_pair, pair, C), _BF16),
            pltpu.VMEM((n_pair, wc, C), _BF16),
            pltpu.VMEM((C, C), _BF16),
            pltpu.VMEM((C, C), _BF16),
            pltpu.VMEM((C, C), _BF16),
            pltpu.VMEM((C // _LANES, 2 * n_q + 8, _LANES), _F32),
            pltpu.SemaphoreType.DMA((1,)),
        ],
        compiler_params=pltpu.CompilerParams(vmem_limit_bytes=96 * 1024 * 1024),
    )(
        c_fine.reshape(n_group, _STRIDE, C),
        p_coarse.reshape(n_group, _STRIDE // 4, C),
        w_lat,
        w_out.reshape(C, C),
    )
    return out.reshape(B, H, W, C)
```

```python
import jax
import jax.numpy as jnp
from jax import lax
import jax.experimental.pallas as pl
import jax.experimental.pallas.tpu as pltpu

_F32 = jnp.float32
_BF16 = jnp.bfloat16
_LANES = 128

_STREAMS = 8
_STRIDE = 4096
_PIECES = (32, 48, 48) * 4
_SWITCH = 17
_INIT = 2
_TAIL = 144


@jax.jit
def pallas_standalone__detection_seg_fpn_lateral__vision_kernel(
    c_fine: jax.Array,
    p_coarse: jax.Array,
    w_lat: jax.Array,
    w_out: jax.Array,
):
    B, H, W, C = c_fine.shape
    assert (B, H, W, C) == (1, 256, 256, 384) and w_out.shape == (1, 1, C, C)
    n_fine = H * W
    pair = 2 * W
    wc = W // 2
    n_pair = n_fine // pair
    n_group = n_fine // _STRIDE
    spg = _STRIDE // pair
    n_slab = n_pair // _STREAMS
    half = _STREAMS // 2
    n_step = 2 * n_slab
    n_q = half * wc
    last = n_step - 1
    sem_p, sem_w, sem_tail = n_step, n_step + n_slab, n_step + n_slab + 2
    n_issued = _INIT + (last - _SWITCH)
    assert sum(_PIECES) == pair
    assert 2 * _INIT <= _SWITCH + 1 and n_issued <= n_slab
    assert all(2 * (i - _SWITCH - 1 + _INIT) + 1 <= i for i in range(_SWITCH + 1, n_step))

    def kernel(c_hbm, p_hbm, wl_hbm, wo_hbm, o_hbm,
               xbuf, pbuf, wl_ref, wo_ref, wf_ref, qup_ref, osem):
        def start_out(sl):
            g0, r0 = (sl // spg) * _STREAMS, (sl % spg) * pair
            lo = 0
            for size in _PIECES:
                pltpu.make_async_copy(
                    xbuf.at[pl.ds(_STREAMS * sl, _STREAMS), pl.ds(lo, size), :],
                    o_hbm.at[pl.ds(g0, _STREAMS), pl.ds(r0 + lo, size), :],
                    osem.at[0]).start()
                lo += size

        def main(rsem):
            def c_in(i, lo=0, size=pair, sem=None):
                sl = i // 2
                g0, r0 = (sl // spg) * _STREAMS + (i % 2) * half, (sl % spg) * pair
                return pltpu.make_async_copy(
                    c_hbm.at[pl.ds(g0, half), pl.ds(r0 + lo, size), :],
                    xbuf.at[pl.ds(half * i, half), pl.ds(lo, size), :],
                    rsem.at[i if sem is None else sem])

            def p_in(sl):
                g0, r0 = (sl // spg) * _STREAMS, (sl % spg) * wc
                return pltpu.make_async_copy(
                    p_hbm.at[pl.ds(g0, _STREAMS), pl.ds(r0, wc), :],
                    pbuf.at[pl.ds(_STREAMS * sl, _STREAMS)],
                    rsem.at[sem_p + sl])

            def c_last_head():
                return c_in(last, 0, pair - _TAIL)

            def c_last_tail():
                return c_in(last, pair - _TAIL, _TAIL, sem_tail)

            wl_in = pltpu.make_async_copy(wl_hbm, wl_ref, rsem.at[sem_w])
            wo_in = pltpu.make_async_copy(wo_hbm, wo_ref, rsem.at[sem_w + 1])
            wl_in.start()
            wo_in.start()
            for i in range(last):
                if i % 2 == 0:
                    p_in(i // 2).start()
                c_in(i).start()
            c_last_head().start()
            c_last_tail().start()

            wl_in.wait()
            wo_in.wait()
            wf_ref[...] = jnp.dot(
                wl_ref[...], wo_ref[...], preferred_element_type=_F32).astype(_BF16)

            def step(i, carry):
                @pl.when(i <= _SWITCH)
                def _():
                    @pl.when(i % 2 == 0)
                    def _():
                        p_in(i // 2).wait()

                    c_in(i).wait()

                rows = pl.ds(half * i, half)
                q = jnp.dot(pbuf[rows].reshape(n_q, C), wo_ref[...],
                            preferred_element_type=_F32)
                for j in range(C // _LANES):
                    qj = q[:, j * _LANES:(j + 1) * _LANES]
                    qup_ref[j, pl.ds(0, n_q, stride=2), :] = qj
                    qup_ref[j, pl.ds(1, n_q, stride=2), :] = qj
                qup = jnp.concatenate(
                    [qup_ref[j, pl.ds(0, 2 * n_q), :] for j in range(C // _LANES)], axis=1)
                y = jnp.dot(xbuf[rows].reshape(half * pair, C), wf_ref[...],
                            preferred_element_type=_F32)
                y = y.reshape(half, 2, W, C) + qup.reshape(half, 1, W, C)
                xbuf[rows] = y.reshape(half, pair, C).astype(_BF16)

                @pl.when(i == _SWITCH)
                def _():
                    for ii in range(_SWITCH + 1, last):
                        if ii % 2 == 0:
                            p_in(ii // 2).wait()
                        c_in(ii).wait()
                    c_last_head().wait()
                    for sl in range(_INIT):
                        start_out(sl)
                    c_last_tail().wait()

                @pl.when(i > _SWITCH)
                def _():
                    start_out(i - (_SWITCH + 1) + _INIT)

                return carry

            lax.fori_loop(0, n_step, step, 0)
            for sl in range(n_issued, n_slab):
                start_out(sl)

        pl.run_scoped(main, pltpu.SemaphoreType.DMA((sem_tail + 1,)))
        pltpu.make_async_copy(o_hbm, o_hbm, osem.at[0]).wait()

    any_spec = pl.BlockSpec(memory_space=pl.ANY)
    out = pl.pallas_call(
        kernel,
        in_specs=[any_spec] * 4,
        out_specs=any_spec,
        out_shape=jax.ShapeDtypeStruct((n_group, _STRIDE, C), _BF16),
        scratch_shapes=[
            pltpu.VMEM((n_pair, pair, C), _BF16),
            pltpu.VMEM((n_pair, wc, C), _BF16),
            pltpu.VMEM((C, C), _BF16),
            pltpu.VMEM((C, C), _BF16),
            pltpu.VMEM((C, C), _BF16),
            pltpu.VMEM((C // _LANES, 2 * n_q + 8, _LANES), _F32),
            pltpu.SemaphoreType.DMA((1,)),
        ],
        compiler_params=pltpu.CompilerParams(vmem_limit_bytes=96 * 1024 * 1024),
    )(
        c_fine.reshape(n_group, _STRIDE, C),
        p_coarse.reshape(n_group, _STRIDE // 4, C),
        w_lat,
        w_out.reshape(C, C),
    )
    return out.reshape(B, H, W, C)
```
